```python
import os as _os
_os.environ.setdefault("JAX_PLATFORMS", "cpu")
import jax
import jax.numpy as jnp

def _softmax(x, axis=-1):
    return jax.nn.softmax(x, axis=axis)
def _gelu(x):
    return jax.nn.gelu(x, approximate=True)
def _silu(x):
    return jax.nn.silu(x)
def _sigmoid(x):
    return jax.nn.sigmoid(x)
def _layernorm(x, axis=-1, eps=1e-5):
    m = jnp.mean(x, axis=axis, keepdims=True)
    v = jnp.var(x, axis=axis, keepdims=True)
    return (x - m) / jnp.sqrt(v + eps)
def _scatter_add(tgt, idx, src, axis=0):
    return tgt.at[idx].add(src)
def _segment_sum(src, seg, n):
    return jax.ops.segment_sum(src, seg, n)
class _Rng:
    def __init__(self, key):
        self._k = key
    def _next(self):
        self._k, sub = jax.random.split(self._k)
        return sub
    def normal(self, shape):
        return jax.random.normal(self._next(), shape, dtype=jnp.bfloat16)
    def randint(self, lo, hi, shape):
        return jax.random.randint(self._next(), shape, lo, hi, dtype=jnp.int32)
    def uniform(self, shape, lo=0.0, hi=1.0):
        return jax.random.uniform(self._next(), shape, jnp.bfloat16, lo, hi)
    def permutation(self, n):
        return jax.random.permutation(self._next(), n)


kernel_name = 'parallel_sum__spectral_gfnet__glu_gated_swiglu__prompt'

def setup_inputs():
    _rng = _Rng(jax.random.key(int.from_bytes(__import__("os").urandom(4), "little")))
    _w = (lambda a: (lambda t: t.astype(jnp.bfloat16) if jnp.issubdtype(t.dtype, jnp.floating) else t)(jnp.asarray(a)))
    def _A_setup():
        B, S, D = 1, 2048, 512
        Df = D // 2 + 1
        return {
            "x": _w((lambda *s: _rng.normal(s) * 0.05)(B, S, D)),
            "w_r": _w((lambda *s: _rng.normal(s) * 0.2)(S, Df) * 0.02),
            "w_i": _w((lambda *s: _rng.normal(s) * 0.2)(S, Df) * 0.02),
        }
    _A_in = _A_setup()

    def _B_setup():
        B, S, D, F = 1, 2048, 512, 1376
        return {
            "x": _w((lambda *s: _rng.normal(s) * 0.05)(B, S, D)),
            "w1": _w((lambda *s: _rng.normal(s) * 0.05)(D, F) * (2.0 / D) ** 0.5),
            "w3": _w((lambda *s: _rng.normal(s) * 0.05)(D, F) * (2.0 / D) ** 0.5),
            "w2": _w((lambda *s: _rng.normal(s) * 0.05)(F, D) * (2.0 / F) ** 0.5),
        }
    _B_in = _B_setup()

    return {
        "A_x": _A_in["x"],
        "A_w_r": _A_in["w_r"],
        "A_w_i": _A_in["w_i"],
        "B_x": _B_in["x"],
        "B_w1": _B_in["w1"],
        "B_w3": _B_in["w3"],
        "B_w2": _B_in["w2"],
    }

def reference(A_x, A_w_r, A_w_i, B_x, B_w1, B_w3, B_w2):
    def _A_ref(x, w_r, w_i):
        B, S, D = x.shape
        X = (lambda x, axes=(-2,-1): jnp.fft.rfft2(x.astype(jnp.float32), axes=axes))(x, axes=(-2, -1))
        W = w_r + 1j * w_i
        X = X * W
        y = (lambda x, s, axes=(-2,-1): jnp.fft.irfft2(x, s=s, axes=axes).astype(jnp.bfloat16))(X, (S, D), axes=(-2, -1))
        return y

    def _B_ref(x, w1, w3, w2):
        gate = jnp.einsum("bsd,df->bsf", x, w1)
        up = jnp.einsum("bsd,df->bsf", x, w3)
        h = _silu(gate) * up
        out = jnp.einsum("bsf,fd->bsd", h, w2)
        return out

    x = A_x
    xn = _layernorm(x, axis=-1)
    return x + _A_ref(xn, A_w_r, A_w_i) + _B_ref(xn, B_w1, B_w3, B_w2)
```

```python
import cmath
import math

import jax
import jax.numpy as jnp
import numpy as np
import jax.experimental.pallas as pl
import jax.experimental.pallas.tpu as pltpu

S, D, F = 2048, 512, 1376
H = D // 2
N1, N2 = 32, 64
TM = 256
NC = S // TM
PS = 40
_NT = (((1,), (1,)), ((), ()))


def _consts():
    d = np.arange(D)[:, None]
    l = np.arange(H)[None, :]
    ang = 2 * np.pi * d * l / D
    fr, fi = np.cos(ang), -np.sin(ang)
    nyq = (-1.0) ** np.arange(D)
    fr[:, 0] = nyq
    fwd = np.stack([np.concatenate([fr[:H, p::2], fi[:H, p::2]], 1) for p in (0, 1)])
    ir, ii = 2 * fr.T / D, 2 * fi.T / D
    ir[0] = nyq / D
    inv = np.stack([np.concatenate([ir[p::2, :H], ii[p::2, :H]], 0) for p in (0, 1)])
    s1 = np.arange(N1)[:, None, None]
    k2 = np.arange(N2)[None, :, None]
    s2 = np.arange(N2)[None, None, :]
    a = -2 * np.pi * ((k2 * (s1 + N1 * s2)) % S) / S
    gr, gi = np.cos(a), np.sin(a)
    g = np.concatenate([np.concatenate([gr, -gi], 2), np.concatenate([gi, gr], 2)], 1)
    gt = g.transpose(0, 2, 1) / S
    bf = jnp.bfloat16
    return fwd.astype(bf), inv.astype(bf), g.astype(bf), gt.astype(bf)


def _tw(v, k, n, sign):
    r, i = v
    if k == 0:
        return v
    if 4 * k == n:
        return (i, -r) if sign < 0 else (-i, r)
    w = cmath.exp(sign * 2j * math.pi * k / n)
    c, s = w.real, w.imag
    if 8 * k == n or 8 * k == 3 * n:
        if c * s > 0:
            return ((r - i) * c, (r + i) * c)
        return ((r + i) * c, (i - r) * c)
    return (r * c - i * s, r * s + i * c)


def _fft(v, sign):
    n = len(v)
    if n == 1:
        return v
    e, o = _fft(v[0::2], sign), _fft(v[1::2], sign)
    lo, hi = [], []
    for k in range(n // 2):
        if 4 * k == n:
            r, i = o[k]
            p, m = (e[k][0] + i, e[k][1] - r), (e[k][0] - i, e[k][1] + r)
            lo.append(p if sign < 0 else m)
            hi.append(m if sign < 0 else p)
            continue
        t = _tw(o[k], k, n, sign)
        lo.append((e[k][0] + t[0], e[k][1] + t[1]))
        hi.append((e[k][0] - t[0], e[k][1] - t[1]))
    return lo + hi


def _kernel(x_h, wr_h, wi_h, w1_h, w3_h, w2_h, fwd_h, inv_h, g_h, gt_h, o_h,
            x_v, wr_v, wi_v, w1_v, w3_v, w2_v, fwd_v, inv_v, g_v, gt_v,
            xn_v, z_v, t_v, o_v, w_v, a_v, sem, wsem, xsem, osem):
    f32, bf = jnp.float32, jnp.bfloat16
    cps = [pltpu.make_async_copy(a, b, sem.at[n]) for n, (a, b) in enumerate(
        [(fwd_h, fwd_v), (g_h, g_v), (gt_h, gt_v),
         (w1_h, w1_v), (w3_h, w3_v), (w2_h, w2_v), (inv_h, inv_v)])]

    def xcp(c):
        r = pl.ds(c * TM, TM)
        return pltpu.make_async_copy(x_h.at[r], x_v.at[r], xsem.at[c])

    def wcp(c):
        r = pl.ds(c * TM, TM)
        return [pltpu.make_async_copy(a.at[:, r], b.at[:, r], wsem.at[n, c])
                for n, (a, b) in enumerate([(wr_h, wr_v), (wi_h, wi_v)])]

    def ocp(c):
        r = pl.ds(c * TM, TM)
        return pltpu.make_async_copy(o_v.at[r], o_h.at[r], osem.at[c])

    xcp(0).start()
    cps[0].start()
    for c in range(NC):
        if c:
            xcp(c).start()
    cps[0].wait()

    def zr(c, m):
        return pl.ds(pl.multiple_of((c * (TM // N1) + m) * PS, 8), N1)

    def zld(t, c):
        return jnp.concatenate([z_v[t, zr(c, m), :].astype(bf) for m in range(TM // N1)], 0)

    def p1(c, _):
        xcp(2 * c).wait()
        xcp(2 * c + 1).wait()

        @pl.when(c == 0)
        def _():
            for n in (1, 3, 4, 5):
                cps[n].start()

        @pl.when(c == 3)
        def _():
            for k in range(NC):
                for w in wcp(k):
                    w.start()
            cps[2].start()
            cps[6].start()
        ln(2 * c)
        ln(2 * c + 1)

    def ln(c):
        r = pl.ds(pl.multiple_of(c * TM, TM), TM)
        x = x_v[r, :].astype(f32)
        xc = x - jnp.mean(x, -1, keepdims=True)
        xn = xc * jax.lax.rsqrt(jnp.mean(xc * xc, -1, keepdims=True) + 1e-5)
        xn_v[r, :] = xn.astype(bf)
        for p, v in enumerate((xn[:, :H] + xn[:, H:], xn[:, :H] - xn[:, H:])):
            z = jnp.dot(v.astype(bf), fwd_v[p], preferred_element_type=f32)
            for t in range(2):
                for m in range(TM // N1):
                    z_v[2 * t + p, zr(c, m), :] = z[m * N1:m * N1 + N1, t * 128:t * 128 + 128]

    def wtr(c):
        r = pl.ds(pl.multiple_of(c * TM, TM), TM)
        row0 = jax.lax.broadcasted_iota(jnp.int32, (H // 2, TM), 0) == 0
        for n, (w, cp) in enumerate(zip((wr_v, wi_v), wcp(c))):
            u = pltpu.bitcast(w[:H, r], jnp.uint32)
            ev = pltpu.bitcast(u << 16, f32)
            od = pltpu.bitcast(u & jnp.uint32(0xFFFF0000), f32)
            ev = jnp.where(row0, w[H:H + 1, r].astype(f32), ev)
            w_v[2 * n, r, :] = ev.T
            w_v[2 * n + 1, r, :] = od.T
    with jax.named_scope("p1"):
        jax.lax.fori_loop(0, NC // 2, p1, None)


    def s1f(j, _):
        z = [z_v[t, pl.ds(j, N2, stride=PS), :].astype(bf) for t in range(4)]
        t_v[j] = jnp.dot(g_v[j], jnp.concatenate([jnp.concatenate(z[:2], 1),
                                                  jnp.concatenate(z[2:], 1)], 0),
                         preferred_element_type=f32)


    def s2f(q, _):
        r0 = pl.multiple_of(q * 8, 8)
        for lt in range(H // 128):
            ls = slice(lt * 128, lt * 128 + 128)
            a, b = pl.ds(r0, 8), pl.ds(r0 + N2, 8)
            v = _fft([(t_v[j, a, ls], t_v[j, b, ls]) for j in range(N1)], -1)
            u = []
            for k, (r, i) in enumerate(v):
                rr = pl.ds(k * N2 + r0, 8)
                p, m = w_v[lt, rr, :], w_v[2 + lt, rr, :]
                u.append((r * p - i * m, r * m + i * p))
            for j, (r, i) in enumerate(_fft(u, 1)):
                t_v[j, a, ls] = r
                t_v[j, b, ls] = i


    def s3f(j, _):
        y = jnp.dot(gt_v[j], t_v[j].astype(bf), preferred_element_type=f32)
        for t in range(4):
            z_v[t, pl.ds(j, N2, stride=PS), :] = y[
                t // 2 * N2:t // 2 * N2 + N2, t % 2 * 128:t % 2 * 128 + 128]


    def ffn(c):
        r = pl.ds(pl.multiple_of(c * TM, TM), TM)
        xn = xn_v[r, :]
        g = jax.lax.dot_general(xn, w1_v[...], _NT, preferred_element_type=f32)
        u = jax.lax.dot_general(xn, w3_v[...], _NT, preferred_element_type=f32)
        h = (g * (0.5 * jnp.tanh(0.5 * g) + 0.5) * u).astype(bf)
        y = jnp.dot(h, w2_v[...], preferred_element_type=f32)
        a_v[r, :] = y + x_v[r, :].astype(f32)

    def fin(c):
        r = pl.ds(pl.multiple_of(c * TM, TM), TM)
        e, o = [jnp.dot(jnp.concatenate([zld(p, c), zld(2 + p, c)], 1),
                        inv_v[p], preferred_element_type=f32) for p in range(2)]
        o_v[r, :] = (a_v[r, :] + jnp.concatenate([e + o, e - o], 1)).astype(bf)
        ocp(c).start()

    def phase(name, c0, fn, k, pre=None, n=2):
        def body(i, _):
            if pre:
                for j in range(k):
                    pre(i * k + j)
            ffn(c0 + i)
            for j in range(k):
                fn(i * k + j)
        with jax.named_scope(name):
            jax.lax.fori_loop(0, n, body, None)

    def wwait(c):
        for w in wcp(c):
            w.wait()

    cps[1].wait()
    with jax.named_scope("s1"):
        jax.lax.fori_loop(0, N1, s1f, None, unroll=8)
    for n in (3, 4, 5):
        cps[n].wait()
    phase("a", 0, wtr, 4, wwait)
    phase("b", 2, lambda q: s2f(q, None), 2, n=4)
    cps[2].wait()
    phase("c", 6, lambda j: s3f(j, None), 32, n=1)
    cps[6].wait()
    with jax.named_scope("d"):
        for c in range(NC - 1):
            fin(c)
        ffn(7)
        fin(7)
    for c in range(NC):
        ocp(c).wait()


@jax.jit
def pallas_parallel_sum__spectral_gfnet__glu_gated_swiglu__prompt_kernel(
        A_x, A_w_r, A_w_i, B_x, B_w1, B_w3, B_w2):
    del B_x
    f32, bf = jnp.float32, jnp.bfloat16
    V = pltpu.VMEM
    hbm = pl.BlockSpec(memory_space=pltpu.HBM)
    out = pl.pallas_call(
        _kernel,
        out_shape=jax.ShapeDtypeStruct((S, D), bf),
        in_specs=[hbm] * 10,
        out_specs=hbm,
        scratch_shapes=[
            V((S, D), bf), V((H + 1, S), bf), V((H + 1, S), bf),
            V((F, D), bf), V((F, D), bf), V((F, D), bf), V((2, H, H), bf), V((2, H, H), bf),
            V((N1, 2 * N2, 2 * N2), bf), V((N1, 2 * N2, 2 * N2), bf),
            V((S, D), bf), V((4, N2 * PS, 128), f32), V((N1, 2 * N2, H), f32), V((S, D), bf),
            V((4, S, 128), f32), V((S, D), f32),
            pltpu.SemaphoreType.DMA((7,)), pltpu.SemaphoreType.DMA((2, NC)), pltpu.SemaphoreType.DMA((NC,)),
            pltpu.SemaphoreType.DMA((NC,)),
        ],
        compiler_params=pltpu.CompilerParams(vmem_limit_bytes=120 * 1024 * 1024),
    )(A_x.reshape(S, D), A_w_r.T, A_w_i.T, B_w1.T, B_w3.T, B_w2, *_consts())
    return out.reshape(1, S, D)
```
